```python
import os as _os
_os.environ.setdefault("JAX_PLATFORMS", "cpu")
import jax
import jax.numpy as jnp

def _softmax(x, axis=-1):
    return jax.nn.softmax(x, axis=axis)
def _gelu(x):
    return jax.nn.gelu(x, approximate=True)
def _silu(x):
    return jax.nn.silu(x)
def _sigmoid(x):
    return jax.nn.sigmoid(x)
def _layernorm(x, axis=-1, eps=1e-5):
    m = jnp.mean(x, axis=axis, keepdims=True)
    v = jnp.var(x, axis=axis, keepdims=True)
    return (x - m) / jnp.sqrt(v + eps)
def _scatter_add(tgt, idx, src, axis=0):
    return tgt.at[idx].add(src)
def _segment_sum(src, seg, n):
    return jax.ops.segment_sum(src, seg, n)
class _Rng:
    def __init__(self, key):
        self._k = key
    def _next(self):
        self._k, sub = jax.random.split(self._k)
        return sub
    def normal(self, shape):
        return jax.random.normal(self._next(), shape, dtype=jnp.bfloat16)
    def randint(self, lo, hi, shape):
        return jax.random.randint(self._next(), shape, lo, hi, dtype=jnp.int32)
    def uniform(self, shape, lo=0.0, hi=1.0):
        return jax.random.uniform(self._next(), shape, jnp.bfloat16, lo, hi)
    def permutation(self, n):
        return jax.random.permutation(self._next(), n)


kernel_name = 'gated_mix__mha_block__dense_activation_mish__prompt'

def setup_inputs():
    _rng = _Rng(jax.random.key(int.from_bytes(__import__("os").urandom(4), "little")))
    _w = (lambda a: (lambda t: t.astype(jnp.bfloat16) if jnp.issubdtype(t.dtype, jnp.floating) else t)(jnp.asarray(a)))
    def _A_setup():
        B, S, D, H = 1, 2048, 640, 32
        return {
            "x": _w((lambda *s: _rng.normal(s) * 0.05)(B, S, D)),
            "wqkv": _w((lambda *s: _rng.normal(s) * 0.2)(D, 3 * D)),
            "wo": _w((lambda *s: _rng.normal(s) * 0.05)(D, D)),
        }
    _A_in = _A_setup()

    def _B_setup():
        B, S, D, F = 1, 2048, 640, 1536
        return {
            "x": _w((lambda *s: _rng.normal(s) * 0.05)(B, S, D)),
            "w1": _w((lambda *s: _rng.normal(s) * 0.8)(D, F) * (D ** -0.5)),
            "b1": _w((lambda *s: _rng.normal(s) * 0.05)(F)),
            "w2": _w((lambda *s: _rng.normal(s) * 0.05)(F, D) * (F ** -0.5)),
        }
    _B_in = _B_setup()

    return {
        "A_x": _A_in["x"],
        "A_wqkv": _A_in["wqkv"],
        "A_wo": _A_in["wo"],
        "B_x": _B_in["x"],
        "B_w1": _B_in["w1"],
        "B_b1": _B_in["b1"],
        "B_w2": _B_in["w2"],
        "gate_w": _w((lambda *s: _rng.normal(s) * 0.05)(640) * 16.0),
    }

def reference(A_x, A_wqkv, A_wo, B_x, B_w1, B_b1, B_w2, gate_w):
    def _A_ref(x, wqkv, wo):
        B, S, D = x.shape
        H = 32
        Dh = D // H
        qkv = (lambda x, *d: x.transpose(*d))((x @ wqkv).reshape(B, S, 3, H, Dh), 2, 0, 3, 1, 4)
        q, k, v = qkv[0], qkv[1], qkv[2]
        scores = jnp.einsum("bhqd,bhkd->bhqk", q, k) * (Dh ** -0.5)
        p = _softmax(scores, axis=-1)
        o = jnp.einsum("bhqk,bhkd->bhqd", p, v)
        return (lambda x, *d: x.transpose(*d))(o, 0, 2, 1, 3).reshape(B, S, D) @ wo

    def _B_ref(x, w1, b1, w2):
        h = jnp.einsum("bsd,df->bsf", x, w1) + b1
        sp = jnp.log1p(jnp.exp(-jnp.abs(h))) + jnp.where(h > 0, h, jnp.zeros_like(h))
        act = h * jnp.tanh(sp)
        return jnp.einsum("bsf,fd->bsd", act, w2)

    x = A_x
    g = _sigmoid((x * gate_w).sum(-1, keepdims=True))
    a = _A_ref(x, A_wqkv, A_wo)
    b = _B_ref(x, B_w1, B_b1, B_w2)
    return g * a + (1 - g) * b
```

```python
import math

import jax
import jax.numpy as jnp
from jax import lax
import jax.experimental.pallas as pl
import jax.experimental.pallas.tpu as pltpu

_S, _D, _H, _DH, _F = 2048, 640, 32, 20, 1536
_NT = (((1,), (1,)), ((), ()))
_LOG2E = 1.4426950408889634
bf16 = jnp.bfloat16
f32 = jnp.float32
u32 = jnp.uint32

TQ = 512
NQB = _S // TQ
NCH = _S // 128


def _kernel(x_ref, wqkv_ref, wo_ref, w1_ref, b1_ref, w2_ref, gw_ref, o_ref,
            q_s, k_s, vt_s, s_s, m_s, ot_s):
    def up(v):
        return pltpu.bitcast(v, bf16)

    R1 = 256
    scale = (_DH ** -0.5) * _LOG2E
    lane1 = lax.broadcasted_iota(jnp.int32, (R1, 128), 1)

    def p1(i, c):
        r0 = pl.multiple_of(i * R1, R1)
        xb = x_ref[pl.ds(r0, R1), :]
        q = jnp.dot(xb, wqkv_ref[:, 0:_D], preferred_element_type=f32) * scale
        k = jnp.dot(xb, wqkv_ref[:, _D:2 * _D], preferred_element_type=f32)
        for b in range(5):
            q_s[b, pl.ds(r0, R1), :] = q[:, b * 128:(b + 1) * 128].astype(bf16)
            k_s[b, pl.ds(r0, R1), :] = k[:, b * 128:(b + 1) * 128].astype(bf16)
        for b, thr in enumerate((120, 112, 124, 116)):
            sel = lane1 >= thr
            q_s[5 + b, pl.ds(r0, R1), :] = jnp.where(
                sel, q[:, b * 128:(b + 1) * 128], q[:, (b + 1) * 128:(b + 2) * 128]).astype(bf16)
            k_s[5 + b, pl.ds(r0, R1), :] = jnp.where(
                sel, k[:, b * 128:(b + 1) * 128], k[:, (b + 1) * 128:(b + 2) * 128]).astype(bf16)
        vt = lax.dot_general(wqkv_ref[:, 2 * _D:3 * _D], xb, (((0,), (1,)), ((), ())),
                             preferred_element_type=f32)
        vt = vt.astype(bf16).astype(f32)
        row = lax.broadcasted_iota(jnp.int32, (24, R1), 0)
        for h in range(_H):
            if h < _H - 1:
                w = vt[h * _DH:h * _DH + 24, :]
            else:
                w = jnp.concatenate([vt[h * _DH:h * _DH + _DH, :], jnp.zeros((4, R1), f32)], axis=0)
            w = jnp.where(row < _DH, w, jnp.where(row == _DH, 1.0, 0.0))
            vt_s[h, :, pl.ds(r0, R1)] = w
        return c

    lax.fori_loop(0, _S // R1, p1, 0)

    qv = q_s.bitcast(u32)
    kv = k_s.bitcast(u32)
    s_s[1] = jnp.zeros((_S, TQ), f32)
    m_s[1] = jnp.zeros((8, TQ), f32)
    lane_q = lax.broadcasted_iota(jnp.int32, (TQ // 2, 128), 1)

    def half(t, sl, do_a=True):
        tp = (t + (_H * NQB - 1)) & (_H * NQB - 1)
        hp = tp >> 2
        qbp = tp & (NQB - 1)
        if do_a:
            h = t >> 2
            qb = t & (NQB - 1)
            c0 = h * _DH
            lo = c0 & 127
            blk = (c0 >> 7) + jnp.where(lo > 128 - _DH, 5, 0)
            qraw = qv[blk, pl.ds(pl.multiple_of(qb * (TQ // 2), TQ // 2), TQ // 2), :]
            q = up(jnp.where(((lane_q - lo) & 127) < _DH, qraw, jnp.uint32(0)))
        mprev = m_s[1 - sl]
        m = None
        acc = jnp.zeros((24, TQ), f32)
        for c in range(NCH):
            if do_a:
                kk = up(kv[blk, c * 64:(c + 1) * 64, :])
                s = lax.dot_general(kk, q, _NT, preferred_element_type=f32)
                s_s[sl, c * 128:(c + 1) * 128, :] = s
                mm = jnp.max(s.reshape(16, 8, TQ), axis=0)
                m = mm if m is None else jnp.maximum(m, mm)
            sp = s_s[1 - sl, c * 128:(c + 1) * 128, :]
            p = jnp.exp2(sp.reshape(16, 8, TQ) - mprev[None]).reshape(128, TQ).astype(bf16)
            v = vt_s[hp, :, c * 128:(c + 1) * 128]
            acc = acc + jnp.dot(v, p, preferred_element_type=f32)
        if do_a:
            m = jnp.maximum(m, pltpu.roll(m, 4, 0))
            m = jnp.maximum(m, pltpu.roll(m, 2, 0))
            m = jnp.maximum(m, pltpu.roll(m, 1, 0))
            m_s[sl] = m
        inv = 1.0 / acc[_DH:_DH + 1, :]
        ot_s[hp, :, pl.ds(pl.multiple_of(qbp * TQ, TQ), TQ)] = acc * inv

    def body(i, c):
        half(2 * i, 0)
        half(2 * i + 1, 1)
        return c

    lax.fori_loop(0, _H * NQB // 2, body, 0)
    half(_H * NQB, 0, do_a=False)

    R3 = 256
    row8 = lax.broadcasted_iota(jnp.int32, (8, R3), 0)
    b1 = b1_ref[...].astype(f32)
    gw = gw_ref[...].astype(f32)

    def p3(i, c):
        r0 = pl.multiple_of(i * R3, R3)
        pieces = []
        for mp in range(_H // 2):
            e = ot_s[2 * mp, :, pl.ds(r0, R3)]
            o = ot_s[2 * mp + 1, :, pl.ds(r0, R3)]
            o0 = pltpu.roll(o[0:8], 4, 0)
            o1 = pltpu.roll(o[8:16], 4, 0)
            o2 = pltpu.roll(o[16:24], 4, 0)
            lowm = row8 < 4
            pieces += [e[0:8], e[8:16], jnp.where(lowm, e[16:24], o0),
                       jnp.where(lowm, o0, o1), jnp.where(lowm, o1, o2)]
        ot = jnp.concatenate(pieces, axis=0)
        ob = ot.T.astype(bf16)
        a = jnp.dot(ob, wo_ref[...], preferred_element_type=f32)
        xb = x_ref[pl.ds(r0, R3), :]
        hh = jnp.dot(xb, w1_ref[...], preferred_element_type=f32) + b1
        n = jnp.exp(jnp.minimum(hh, 20.0))
        tt = n * (n + 2.0)
        act = (hh * (tt / (tt + 2.0))).astype(bf16)
        b = jnp.dot(act, w2_ref[...], preferred_element_type=f32)
        gl = jnp.sum(xb.astype(f32) * gw, axis=1, keepdims=True)
        g = 1.0 / (1.0 + jnp.exp(-gl))
        o_ref[pl.ds(r0, R3), :] = (g * a + (1.0 - g) * b).astype(o_ref.dtype)
        return c

    lax.fori_loop(0, _S // R3, p3, 0)


@jax.jit
def pallas_gated_mix__mha_block__dense_activation_mish__prompt_kernel(
    A_x, A_wqkv, A_wo, B_x, B_w1, B_b1, B_w2, gate_w,
):
    del B_x
    x = A_x.reshape(_S, _D)
    out = pl.pallas_call(
        _kernel,
        out_shape=jax.ShapeDtypeStruct((_S, _D), A_x.dtype),
        scratch_shapes=[
            pltpu.VMEM((9, _S, 128), bf16),
            pltpu.VMEM((9, _S, 128), bf16),
            pltpu.VMEM((_H, 24, _S), f32),
            pltpu.VMEM((2, _S, TQ), f32),
            pltpu.VMEM((2, 8, TQ), f32),
            pltpu.VMEM((_H, 24, _S), f32),
        ],
        compiler_params=pltpu.CompilerParams(vmem_limit_bytes=100 * 1024 * 1024),
    )(x, A_wqkv, A_wo, B_w1, B_b1.reshape(1, _F), B_w2, gate_w.reshape(1, _D))
    return out.reshape(1, _S, _D)
```

```python
import jax
import jax.numpy as jnp
from jax import lax
import jax.experimental.pallas as pl
import jax.experimental.pallas.tpu as pltpu

_S, _D, _H, _DH, _F = 2048, 640, 32, 20, 1536
_NT = (((1,), (1,)), ((), ()))
_TN = (((0,), (1,)), ((), ()))
_LOG2E = 1.4426950408889634

_TQ = 512
_NQB = _S // _TQ
_NCH = _S // 128
_R = 256
_NB = _S // _R
_HEADS_PER_ITER = 2


def _kernel(x_hbm, wqkv_hbm, wo_hbm, w1_hbm, b1_hbm, w2_hbm, gw_hbm, o_hbm,
            q_s, k_s, vt_s, s_s, m_s, ot_s,
            x_ref, wqkv_ref, wo_ref, w1_ref, b1_ref, w2_ref, gw_ref, o_ref,
            sem_x, sem_w, sem_o):
    bf16, f32, u32 = jnp.bfloat16, jnp.float32, jnp.uint32

    def x_copy(i):
        rows = pl.ds(i * _R, _R)
        return pltpu.make_async_copy(x_hbm.at[rows, :], x_ref.at[rows, :], sem_x.at[i])

    def o_copy(i):
        rows = pl.ds(i * _R, _R)
        return pltpu.make_async_copy(o_ref.at[rows, :], o_hbm.at[rows, :], sem_o.at[i])

    def wqkv_copy(j):
        cols = pl.ds(j * _D, _D)
        return pltpu.make_async_copy(wqkv_hbm.at[:, cols], wqkv_ref.at[:, cols], sem_w.at[j])

    late = [pltpu.make_async_copy(src, dst, sem_w.at[3 + j]) for j, (src, dst) in enumerate(
        ((w1_hbm, w1_ref), (w2_hbm, w2_ref), (wo_hbm, wo_ref),
         (b1_hbm, b1_ref), (gw_hbm, gw_ref)))]

    x_copy(0).start()
    wqkv_copy(1).start()
    wqkv_copy(0).start()
    s_s[1] = jnp.zeros((_S, _TQ), f32)
    m_s[1] = jnp.zeros((8, _TQ), f32)

    q_scale = (_DH ** -0.5) * _LOG2E
    lane = lax.broadcasted_iota(jnp.int32, (_R, 128), 1)
    row24 = lax.broadcasted_iota(jnp.int32, (24, _R), 0)

    def store_lane_blocks(dst, val, r0):
        for b in range(5):
            dst[b, pl.ds(r0, _R), :] = val[:, b * 128:(b + 1) * 128].astype(bf16)
        for b, first in enumerate((120, 112, 124, 116)):
            dst[5 + b, pl.ds(r0, _R), :] = jnp.where(
                lane >= first, val[:, b * 128:(b + 1) * 128],
                val[:, (b + 1) * 128:(b + 2) * 128]).astype(bf16)

    def project(r0, before=(None, None, None)):
        if before[0] is not None:
            before[0]()
        xb = x_ref[pl.ds(r0, _R), :]
        k = jnp.dot(xb, wqkv_ref[:, _D:2 * _D], preferred_element_type=f32)
        store_lane_blocks(k_s, k, r0)
        if before[1] is not None:
            before[1]()
        q = jnp.dot(xb, wqkv_ref[:, 0:_D], preferred_element_type=f32) * q_scale
        store_lane_blocks(q_s, q, r0)
        if before[2] is not None:
            before[2]()
        vt = lax.dot_general(wqkv_ref[:, 2 * _D:3 * _D], xb, _TN, preferred_element_type=f32)
        vt = vt.astype(bf16).astype(f32)
        for h in range(_H):
            if h < _H - 1:
                w = vt[h * _DH:h * _DH + 24, :]
            else:
                w = jnp.concatenate([vt[h * _DH:, :], jnp.zeros((4, _R), f32)], axis=0)
            vt_s[h, :, pl.ds(r0, _R)] = jnp.where(
                row24 < _DH, w, jnp.where(row24 == _DH, 1.0, 0.0))

    def before_k():
        x_copy(0).wait()
        wqkv_copy(1).wait()
        wqkv_copy(2).start()

    def before_q():
        x_copy(1).start()
        x_copy(2).start()
        wqkv_copy(0).wait()

    def before_v():
        wqkv_copy(2).wait()
        for i in range(3, _NB):
            x_copy(i).start()

    project(0, (before_k, before_q, before_v))
    for cpy in late:
        cpy.start()

    def project_step(i, carry):
        x_copy(i).wait()
        project(pl.multiple_of(i * _R, _R))
        return carry

    lax.fori_loop(1, _NB, project_step, 0)
    for cpy in late:
        cpy.wait()

    q32 = q_s.bitcast(u32)
    k32 = k_s.bitcast(u32)
    lane_q = lax.broadcasted_iota(jnp.int32, (_TQ // 2, 128), 1)

    def step(h, qb, slot, with_scores=True):
        if qb > 0:
            hp, qbp = h, qb - 1
        else:
            hp, qbp = (h + (_H - 1)) & (_H - 1), _NQB - 1
        if with_scores:
            col = h * _DH
            first = col & 127
            blk = (col >> 7) + jnp.where(first > 128 - _DH, 5, 0)
            qraw = q32[blk, qb * (_TQ // 2):(qb + 1) * (_TQ // 2), :]
            q = pltpu.bitcast(
                jnp.where(((lane_q - first) & 127) < _DH, qraw, jnp.uint32(0)), bf16)
        m_prev = m_s[1 - slot]
        m = None
        acc = jnp.zeros((24, _TQ), f32)
        for c in range(_NCH):
            keys = slice(c * 128, (c + 1) * 128)
            if with_scores:
                kc = pltpu.bitcast(k32[blk, c * 64:(c + 1) * 64, :], bf16)
                s = lax.dot_general(kc, q, _NT, preferred_element_type=f32)
                s_s[slot, keys, :] = s
                mc = jnp.max(s.reshape(16, 8, _TQ), axis=0)
                m = mc if m is None else jnp.maximum(m, mc)
            sp = s_s[1 - slot, keys, :]
            p = jnp.exp2(sp.reshape(16, 8, _TQ) - m_prev[None]).reshape(128, _TQ)
            acc = acc + jnp.dot(vt_s[hp, :, keys], p.astype(bf16), preferred_element_type=f32)
        if with_scores:
            for shift in (4, 2, 1):
                m = jnp.maximum(m, pltpu.roll(m, shift, 0))
            m_s[slot] = m
        denom = acc[_DH:_DH + 1, :]
        inv = pltpu.reciprocal(denom, approx=True)
        inv = inv * (2.0 - denom * inv)
        ot_s[hp, :, qbp * _TQ:(qbp + 1) * _TQ] = acc * inv

    def attention_step(i, carry):
        for u in range(_HEADS_PER_ITER * _NQB):
            step(_HEADS_PER_ITER * i + u // _NQB, u % _NQB, u & 1)
        return carry

    lax.fori_loop(0, _H // _HEADS_PER_ITER, attention_step, 0)
    step(_H, 0, 0, with_scores=False)

    low4 = lax.broadcasted_iota(jnp.int32, (8, _R), 0) < 4
    b1 = b1_ref[...].astype(f32)
    b1 = jnp.concatenate([b1[j:j + 1, :] for j in range(_F // 128)], axis=1)
    gw = gw_ref[...].astype(f32)
    gw = jnp.concatenate([gw[j:j + 1, :] for j in range(_D // 128)], axis=1)

    def finish(i, r0):
        xb = x_ref[pl.ds(r0, _R), :]
        hid = jnp.dot(xb, w1_ref[...], preferred_element_type=f32) + b1
        pieces = []
        for pair in range(_H // 2):
            e = ot_s[2 * pair, :, pl.ds(r0, _R)]
            o = ot_s[2 * pair + 1, :, pl.ds(r0, _R)]
            o0, o1, o2 = (pltpu.roll(o[8 * j:8 * j + 8], 4, 0) for j in range(3))
            pieces += [e[0:8], e[8:16], jnp.where(low4, e[16:24], o0),
                       jnp.where(low4, o0, o1), jnp.where(low4, o1, o2)]
        att = jnp.concatenate(pieces, axis=0).T.astype(bf16)
        a = jnp.dot(att, wo_ref[...], preferred_element_type=f32)
        n = jnp.exp(jnp.minimum(hid, 20.0))
        t = n * (n + 2.0)
        den = t + 2.0
        r = pltpu.reciprocal(den, approx=True)
        r = r * (2.0 - den * r)
        act = (hid * (t * r)).astype(bf16)
        b = jnp.dot(act, w2_ref[...], preferred_element_type=f32)
        logit = jnp.sum(xb.astype(f32) * gw, axis=1, keepdims=True)
        g = 1.0 / (1.0 + jnp.exp(-logit))
        o_ref[pl.ds(r0, _R), :] = (b + g * (a - b)).astype(o_ref.dtype)
        o_copy(i).start()

    def finish_step(i, carry):
        finish(i, pl.multiple_of(i * _R, _R))
        return carry

    finish(0, 0)
    lax.fori_loop(1, _NB, finish_step, 0)
    for i in range(_NB):
        o_copy(i).wait()


@jax.jit
def pallas_gated_mix__mha_block__dense_activation_mish__prompt_kernel(
    A_x: jax.Array,
    A_wqkv: jax.Array,
    A_wo: jax.Array,
    B_x: jax.Array,
    B_w1: jax.Array,
    B_b1: jax.Array,
    B_w2: jax.Array,
    gate_w: jax.Array,
):
    del B_x
    bf16, f32 = jnp.bfloat16, jnp.float32
    out = pl.pallas_call(
        _kernel,
        out_shape=jax.ShapeDtypeStruct((_S, _D), A_x.dtype),
        in_specs=[pl.BlockSpec(memory_space=pl.ANY)] * 7,
        out_specs=pl.BlockSpec(memory_space=pl.ANY),
        scratch_shapes=[
            pltpu.VMEM((9, _S, 128), bf16),
            pltpu.VMEM((9, _S, 128), bf16),
            pltpu.VMEM((_H, 24, _S), f32),
            pltpu.VMEM((2, _S, _TQ), f32),
            pltpu.VMEM((2, 8, _TQ), f32),
            pltpu.VMEM((_H, 24, _S), f32),
            pltpu.VMEM((_S, _D), bf16),
            pltpu.VMEM((_D, 3 * _D), bf16),
            pltpu.VMEM((_D, _D), bf16),
            pltpu.VMEM((_D, _F), bf16),
            pltpu.VMEM((_F // 128, 128), bf16),
            pltpu.VMEM((_F, _D), bf16),
            pltpu.VMEM((_D // 128, 128), bf16),
            pltpu.VMEM((_S, _D), bf16),
            pltpu.SemaphoreType.DMA((_NB,)),
            pltpu.SemaphoreType.DMA((8,)),
            pltpu.SemaphoreType.DMA((_NB,)),
        ],
        compiler_params=pltpu.CompilerParams(vmem_limit_bytes=100 * 1024 * 1024),
    )(A_x.reshape(_S, _D), A_wqkv, A_wo, B_w1, B_b1.reshape(_F // 128, 128), B_w2,
      gate_w.reshape(_D // 128, 128))
    return out.reshape(1, _S, _D)
```
